```python
import jax
import jax.numpy as jnp

def _softmax(x, axis=-1):
    return jax.nn.softmax(x, axis=axis)
def _gelu(x):
    return jax.nn.gelu(x, approximate=True)
def _silu(x):
    return jax.nn.silu(x)
def _sigmoid(x):
    return jax.nn.sigmoid(x)
def _layernorm(x, axis=-1, eps=1e-5):
    m = jnp.mean(x, axis=axis, keepdims=True)
    v = jnp.var(x, axis=axis, keepdims=True)
    return (x - m) / jnp.sqrt(v + eps)
def _scatter_add(tgt, idx, src, axis=0):
    return tgt.at[idx].add(src)
def _segment_sum(src, seg, n):
    return jax.ops.segment_sum(src, seg, n)
class _Rng:
    def __init__(self, key):
        self._k = key
    def _next(self):
        self._k, sub = jax.random.split(self._k)
        return sub
    def normal(self, shape):
        return jax.random.normal(self._next(), shape, dtype=jnp.bfloat16)
    def randint(self, lo, hi, shape):
        return jax.random.randint(self._next(), shape, lo, hi, dtype=jnp.int32)
    def uniform(self, shape, lo=0.0, hi=1.0):
        return jax.random.uniform(self._next(), shape, jnp.bfloat16, lo, hi)
    def permutation(self, n):
        return jax.random.permutation(self._next(), n)


kernel_name = 'sequential_preLN__grouped_kv_mqa__glu_gated_swiglu__prompt'

def _fwd_setup_inputs():
    _rng = _Rng(jax.random.key(int.from_bytes(__import__("os").urandom(4), "little")))
    _w = (lambda a: (lambda t: t.astype(jnp.bfloat16) if jnp.issubdtype(t.dtype, jnp.floating) else t)(jnp.asarray(a)))
    def _A_setup():
        B, S, D, H = 1, 2048, 512, 32
        Dh = D // H
        return {
            "x": _w((lambda *s: _rng.normal(s) * 0.05)(B, S, D)),
            "wq": _w((lambda *s: _rng.normal(s) * 0.05)(D, H * Dh)),
            "wk": _w((lambda *s: _rng.normal(s) * 0.05)(D, Dh)),
            "wv": _w((lambda *s: _rng.normal(s) * 0.05)(D, Dh)),
            "wo": _w((lambda *s: _rng.normal(s) * 0.05)(H * Dh, D)),
        }
    _A_in = _A_setup()

    def _B_setup():
        B, S, D, F = 1, 2048, 512, 1376
        return {
            "x": _w((lambda *s: _rng.normal(s) * 0.05)(B, S, D)),
            "w1": _w((lambda *s: _rng.normal(s) * 0.05)(D, F) * (2.0 / D) ** 0.5),
            "w3": _w((lambda *s: _rng.normal(s) * 0.05)(D, F) * (2.0 / D) ** 0.5),
            "w2": _w((lambda *s: _rng.normal(s) * 0.05)(F, D) * (2.0 / F) ** 0.5),
        }
    _B_in = _B_setup()

    return {
        "A_x": _A_in["x"],
        "A_wq": _A_in["wq"],
        "A_wk": _A_in["wk"],
        "A_wv": _A_in["wv"],
        "A_wo": _A_in["wo"],
        "B_x": _B_in["x"],
        "B_w1": _B_in["w1"],
        "B_w3": _B_in["w3"],
        "B_w2": _B_in["w2"],
    }

def _fwd_reference(A_x, A_wq, A_wk, A_wv, A_wo, B_x, B_w1, B_w3, B_w2):
    def _A_ref(x, wq, wk, wv, wo):
        B, S, D = x.shape
        H = 32
        Dh = D // H
        q = (lambda x, *d: x.transpose(*d))((x @ wq).reshape(B, S, H, Dh), 0, 2, 1, 3)
        k = x @ wk
        v = x @ wv
        scores = jnp.einsum("bhqd,bkd->bhqk", q, k) * (Dh ** -0.5)
        p = _softmax(scores, axis=-1)
        o = jnp.einsum("bhqk,bkd->bhqd", p, v)
        return (lambda x, *d: x.transpose(*d))(o, 0, 2, 1, 3).reshape(B, S, H * Dh) @ wo

    def _B_ref(x, w1, w3, w2):
        gate = jnp.einsum("bsd,df->bsf", x, w1)
        up = jnp.einsum("bsd,df->bsf", x, w3)
        h = _silu(gate) * up
        out = jnp.einsum("bsf,fd->bsd", h, w2)
        return out

    x = A_x
    h = x + _A_ref(_layernorm(x, axis=-1), A_wq, A_wk, A_wv, A_wo)
    h2 = h + _B_ref(_layernorm(h, axis=-1), B_w1, B_w3, B_w2)
    return h2


def setup_inputs():
    _inp = _fwd_setup_inputs()
    _gk = jax.random.fold_in(jax.random.key(int.from_bytes(__import__("os").urandom(4), "little")), 2**31 - 1)
    _shapes = [[1, 2048, 512]]
    _dtypes = ['bfloat16']
    _gks = jax.random.split(_gk, len(_shapes))
    _gs = [jax.random.normal(k, s, dtype=jnp.dtype(d)) * 0.05 for k, s, d in zip(_gks, _shapes, _dtypes)]
    _inp["grad_out"] = _gs[0]
    return _inp

def reference(A_x, A_wq, A_wk, A_wv, A_wo, B_w1, B_w3, B_w2, B_x, grad_out):
    _const = dict(B_x=B_x)
    def _f(*_d):
        return _fwd_reference(**{'A_x': _d[0], 'A_wq': _d[1], 'A_wk': _d[2], 'A_wv': _d[3], 'A_wo': _d[4], 'B_w1': _d[5], 'B_w3': _d[6], 'B_w2': _d[7], **_const})
    _out, _vjp = jax.vjp(_f, A_x, A_wq, A_wk, A_wv, A_wo, B_w1, B_w3, B_w2)
    _grads = _vjp(grad_out)
    _out0 = jnp.asarray(_out)
    return (_out0, *[jnp.asarray(_g) for _g in _grads])
```

```python
import functools
import math

import jax
import jax.numpy as jnp
from jax import lax
import jax.experimental.pallas as pl
import jax.experimental.pallas.tpu as pltpu

S = 2048
D = 512
H = 32
DH = 16
F = 1376
EPS = 1e-5

T = 128
HPI_F = 8
HPI_B = 8
LAG_F = 2
LAG_B = 2
KC = 512
SAFE_BOUND = 40.0

LOG2E = 1.4426950408889634
LN2 = 0.6931471805599453
QSCALE = (DH ** -0.5) * LOG2E

bf = jnp.bfloat16
f32 = jnp.float32
NT = (((1,), (1,)), ((), ()))
TN = (((0,), (0,)), ((), ()))


def _tobf(x):
    return pltpu.bitcast(x, bf)


def _tou(x):
    return pltpu.bitcast(x, jnp.uint32)


def _mm(a, b):
    return jnp.dot(a, b, preferred_element_type=f32)


def _mm_nt(a, b):
    return lax.dot_general(a, b, NT, preferred_element_type=f32)


def _mm_tn(a, b):
    return lax.dot_general(a, b, TN, preferred_element_type=f32)


def _ln(x):
    mu = jnp.mean(x, axis=-1, keepdims=True)
    xc = x - mu
    var = jnp.mean(xc * xc, axis=-1, keepdims=True)
    rstd = lax.rsqrt(var + EPS)
    return xc * rstd, rstd


def _ln_bwd(dy, y, rstd):
    m1 = jnp.mean(dy, axis=-1, keepdims=True)
    m2 = jnp.mean(dy * y, axis=-1, keepdims=True)
    return rstd * (dy - m1 - y * m2)


def _split3(v):
    hi = v.astype(bf).astype(f32)
    r = v - hi
    mid = r.astype(bf).astype(f32)
    lo = (r - mid).astype(bf).astype(f32)
    return hi, mid, lo


def _ext_rows(a, b, c):
    row = lax.broadcasted_iota(jnp.int32, (16, 128), 0)
    z = jnp.zeros((16, 128), f32)
    return jnp.where(row == 0, a, jnp.where(row == 1, b, jnp.where(row == 2, c, z)))


def _make_kernel(T, hpi_f, hpi_b, lag_f, lag_b):
    NQ = T // 128
    NBLK = S // T
    NC = S // KC

    def build_stack(stack_ref, main_fn, ext_fn):
        for t in range(NQ):
            for g4 in range(H // 4):
                parts = []
                for i in range(4):
                    h = 4 * g4 + i
                    parts.append(main_fn(h, t))
                    parts.append(ext_fn(h, t))
                tile = jnp.concatenate(parts, axis=0).astype(bf)
                tt = _tou(tile.T)
                for i in range(4):
                    h = 4 * g4 + i
                    r = tt if i == 0 else pltpu.roll(tt, 128 - 32 * i, 1)
                    stack_ref[h * NQ + t] = r

    def kernel(x_ref, wq_ref, wk_ref, wv_ref, wo_ref, w1_ref, w3_ref, w2_ref, g_ref,
               out_ref, dx_ref, dwq_ref, dwk_ref, dwv_ref, dwo_ref, dw1_ref, dw3_ref, dw2_ref,
               xn_s, wqT_s, ktext_s, vtext_s, qstack_s, qT_s, dostack_s, doT_s, p_s, ds_s,
               oT_s, linv_s, dqT_s, dkT_s, dvT_s,
               dwqT_acc, dwo_acc, dw1_acc, dw3_acc, dw2_acc, dxp_s, kmax_s):
        step = pl.program_id(0)

        @pl.when(step == 0)
        def _prologue():
            def ln_chunk(i, c):
                r = pl.ds(pl.multiple_of(i * 256, 256), 256)
                xn, _ = _ln(x_ref[r, :].astype(f32))
                xn_s[r, :] = xn.astype(bf)
                return c
            lax.fori_loop(0, S // 256, ln_chunk, 0)
            wqT_s[...] = wq_ref[...].T
            xn_all = xn_s[...]
            dn = (((0,), (1,)), ((), ()))
            kT = lax.dot_general(wk_ref[...], xn_all, dn, preferred_element_type=f32).astype(bf)
            vT = lax.dot_general(wv_ref[...], xn_all, dn, preferred_element_type=f32).astype(bf)
            row = lax.broadcasted_iota(jnp.int32, (16, S), 0)
            ones3 = jnp.where(row < 3, 1.0, 0.0).astype(bf)
            ktext_s[...] = _tou(jnp.concatenate([kT, ones3], axis=0))
            vtext_s[...] = _tou(jnp.concatenate([vT, ones3], axis=0))
            kf = kT.astype(f32)
            k2 = jnp.sum(kf * kf, axis=0, keepdims=True)
            kmax_s[0] = jnp.max(k2)
            for r in (dwqT_acc, dwo_acc, dw1_acc, dw3_acc, dw2_acc, dkT_s, dvT_s):
                r[...] = jnp.zeros_like(r)

        rows = pl.ds(pl.multiple_of(step * T, T), T)

        xn_b = xn_s[rows, :]
        qT = _mm_nt(wqT_s[...], xn_b) * QSCALE
        qTb = qT.astype(bf)
        qT_s[...] = _tou(qTb)
        qTr = qTb.astype(f32)
        sq = qTr * qTr
        n2 = jnp.sum(sq[0:16], axis=0, keepdims=True)
        for h in range(1, H):
            n2 = jnp.maximum(n2, jnp.sum(sq[16 * h:16 * h + 16], axis=0, keepdims=True))
        b2 = jnp.max(n2) * kmax_s[0]
        safe = b2 <= SAFE_BOUND * SAFE_BOUND
        mvec = jnp.sqrt(jnp.full((1, 128), b2, f32)) * 1.01
        mvec = jnp.where(jnp.full((1, 128), b2, f32) <= SAFE_BOUND * SAFE_BOUND, mvec, 0.0)
        zrow = jnp.zeros((1, 128), f32)
        ext_q = _ext_rows(-mvec, zrow, zrow)
        build_stack(qstack_s,
                    lambda h, t: qT[16 * h:16 * h + 16, t * 128:(t + 1) * 128],
                    lambda h, t: ext_q)

        @pl.when(jnp.logical_not(safe))
        def _true_max():
            def body(i, c):
                lhs = _tobf(qstack_s[i])[:, 0:32]
                m = None
                for cc in range(NC):
                    s = _mm(lhs, _tobf(ktext_s[:, cc * KC:(cc + 1) * KC]))
                    mc = jnp.max(s, axis=1, keepdims=True)
                    m = mc if m is None else jnp.maximum(m, mc)
                hi, mid, lo = _split3(-m)
                lane = lax.broadcasted_iota(jnp.int32, (128, 128), 1)
                cur = _tobf(qstack_s[i]).astype(f32)
                new = jnp.where(lane == 16, hi, jnp.where(lane == 17, mid, jnp.where(lane == 18, lo, cur)))
                qstack_s[i] = _tou(new.astype(bf))
                return c
            lax.fori_loop(0, H * NQ, body, 0)

        def fwd_body(it, carry):
            its = [(it * hpi_f * NQ + j, c) for j in range(hpi_f * NQ) for c in range(NC)]
            acc, lacc = {}, {}

            def s_part(n):
                i, c = its[n]
                ks = slice(c * KC, (c + 1) * KC)
                s = _mm(_tobf(qstack_s[i])[:, 0:32], _tobf(ktext_s[:, ks]))
                p = jnp.exp2(s)
                ps = p[:, 0:128]
                for j in range(1, KC // 128):
                    ps = ps + p[:, j * 128:(j + 1) * 128]
                k = n // NC
                lacc[k] = ps if c == 0 else lacc[k] + ps
                p_s[i, :, ks] = _tou(p.astype(bf))

            def pv(n):
                i, c = its[n]
                ks = slice(c * KC, (c + 1) * KC)
                r = _mm_nt(_tobf(vtext_s[0:8, ks]), _tobf(p_s[i, :, ks]))
                k = n // NC
                acc[k] = r if c == 0 else acc[k] + r
                if c == NC - 1:
                    l = jnp.sum(lacc[k].T, axis=0, keepdims=True)
                    linv = 1.0 / l
                    oT_s[i] = acc[k] * linv
                    linv_s[i] = linv

            N = len(its)
            for n in range(N + lag_f):
                if n < N:
                    s_part(n)
                if n >= lag_f:
                    pv(n - lag_f)
            return carry
        lax.fori_loop(0, H // hpi_f, fwd_body, 0)

        oT = jnp.concatenate(
            [jnp.concatenate([oT_s[h * NQ + t] for t in range(NQ)], axis=1) if NQ > 1 else oT_s[h]
             for h in range(H)], axis=0)
        oTb = oT.astype(bf)
        o_b = oTb.T
        x_b = x_ref[rows, :].astype(f32)
        hres = x_b + _mm(o_b, wo_ref[...])
        hn, rstd_h = _ln(hres)
        hn_b = hn.astype(bf)
        gate = _mm(hn_b, w1_ref[...])
        up = _mm(hn_b, w3_ref[...])
        sig = jax.nn.sigmoid(gate)
        silu = gate * sig
        act_b = (silu * up).astype(bf)
        out_ref[...] = (hres + _mm(act_b, w2_ref[...])).astype(out_ref.dtype)

        dy_b = g_ref[...]
        dact = _mm_nt(dy_b, w2_ref[...])
        dw2_acc[...] += _mm_tn(act_b, dy_b)
        dgate_b = (dact * up * (sig * (1.0 + gate * (1.0 - sig)))).astype(bf)
        dup_b = (dact * silu).astype(bf)
        dhn = _mm_nt(dgate_b, w1_ref[...]) + _mm_nt(dup_b, w3_ref[...])
        hnT_b = hn_b.T
        dw1_acc[...] += _mm(hnT_b, dgate_b)
        dw3_acc[...] += _mm(hnT_b, dup_b)
        dh = dy_b.astype(f32) + _ln_bwd(dhn, hn, rstd_h)
        dh_b = dh.astype(bf)
        dwo_acc[...] += _mm(oTb, dh_b)
        doT = _mm_nt(wo_ref[...], dh_b)

        dos = {}
        dlt = {}
        for h in range(H):
            for t in range(NQ):
                cs = slice(t * 128, (t + 1) * 128)
                d = (doT[16 * h:16 * h + 16, cs] * linv_s[h * NQ + t]).astype(bf)
                df = d.astype(f32)
                dos[h, t] = df
                dl = jnp.sum(df * oT[16 * h:16 * h + 16, cs], axis=0, keepdims=True)
                dlt[h, t] = _ext_rows(*_split3(-dl))
        doT_rows = [jnp.concatenate([dos[h, t] for t in range(NQ)], axis=1) if NQ > 1 else dos[h, 0]
                    for h in range(H)]
        doT_s[...] = _tou(jnp.concatenate(doT_rows, axis=0).astype(bf))
        build_stack(dostack_s, lambda h, t: dos[h, t], lambda h, t: dlt[h, t])

        def bwd_body(it, carry):
            its = [(it * hpi_b * NQ + j, c) for j in range(hpi_b * NQ) for c in range(NC)]
            acc = {}

            def dp_part(n):
                i, c = its[n]
                ks = slice(c * KC, (c + 1) * KC)
                dp = _mm(_tobf(dostack_s[i])[:, 0:32], _tobf(vtext_s[:, ks]))
                ds = _tobf(p_s[i, :, ks]).astype(f32) * dp
                ds_s[n] = _tou(ds.astype(bf))

            def small(n):
                i, c = its[n]
                ks = slice(c * KC, (c + 1) * KC)
                j = n // NC
                hh = it * hpi_b + j // NQ
                t = j % NQ
                hr = pl.ds(pl.multiple_of(hh * 8, 8), 8)
                r = _mm_nt(_tobf(ktext_s[0:8, ks]), _tobf(ds_s[n]))
                acc[j] = r if c == 0 else acc[j] + r
                if c == NC - 1:
                    dqT_s[i] = acc[j]
                dkT_s[:, ks] += _mm(_tobf(qT_s[hr, t * 128:(t + 1) * 128]), _tobf(ds_s[n]))
                dvT_s[:, ks] += _mm(_tobf(doT_s[hr, t * 128:(t + 1) * 128]), _tobf(p_s[i, :, ks]))

            N = len(its)
            for n in range(N + lag_b):
                if n < N:
                    dp_part(n)
                if n >= lag_b:
                    small(n - lag_b)
            return carry
        lax.fori_loop(0, H // hpi_b, bwd_body, 0)

        dqT = jnp.concatenate(
            [jnp.concatenate([dqT_s[h * NQ + t] for t in range(NQ)], axis=1) if NQ > 1 else dqT_s[h]
             for h in range(H)], axis=0) * (DH ** -0.5)
        dqT_b = dqT.astype(bf)
        dwqT_acc[...] += _mm(dqT_b, xn_b)
        dxnT = _mm(wq_ref[...], dqT_b)
        dxn = dxnT.T
        xn_f, rstd_x = _ln(x_b)
        dxp_s[rows, :] = dh + _ln_bwd(dxn, xn_f, rstd_x)

        @pl.when(step == NBLK - 1)
        def _epilogue():
            dkT = dkT_s[...] * LN2
            dvT = dvT_s[...]
            dkvT_b = jnp.concatenate([dkT, dvT], axis=0).astype(bf)
            xn_all = xn_s[...]
            dwkvT = _mm(dkvT_b, xn_all)
            pad = jnp.concatenate([dwkvT, jnp.zeros((96, D), f32)], axis=0)
            dwkv = pad.T
            dwk_ref[...] = dwkv[:, 0:16].astype(dwk_ref.dtype)
            dwv_ref[...] = dwkv[:, 16:32].astype(dwv_ref.dtype)
            dn = (((0,), (1,)), ((), ()))

            def chunk(i, c):
                o = pl.multiple_of(i * 256, 256)
                r = pl.ds(o, 256)
                dk_c = dkT_s[:, r] * LN2
                dxk = lax.dot_general(dk_c.astype(bf), wk_ref[...], dn, preferred_element_type=f32)
                dxv = lax.dot_general(dvT_s[:, r].astype(bf), wv_ref[...], dn, preferred_element_type=f32)
                xn_f, rstd_x = _ln(x_ref[r, :].astype(f32))
                dx_ref[r, :] = (dxp_s[r, :] + _ln_bwd(dxk + dxv, xn_f, rstd_x)).astype(dx_ref.dtype)
                return c
            lax.fori_loop(0, S // 256, chunk, 0)
            dwq_ref[...] = dwqT_acc[...].T.astype(dwq_ref.dtype)
            dwo_ref[...] = dwo_acc[...].astype(dwo_ref.dtype)
            dw1_ref[...] = dw1_acc[...].astype(dw1_ref.dtype)
            dw3_ref[...] = dw3_acc[...].astype(dw3_ref.dtype)
            dw2_ref[...] = dw2_acc[...].astype(dw2_ref.dtype)

    return kernel


def _call(A_x, A_wq, A_wk, A_wv, A_wo, B_w1, B_w3, B_w2, grad_out,
          T=T, hpi_f=HPI_F, hpi_b=HPI_B, lag_f=LAG_F, lag_b=LAG_B):
    NQ = T // 128
    NC = S // KC
    x2 = A_x.reshape(S, D)
    g2 = grad_out.reshape(S, D)

    def res(shape):
        return pl.BlockSpec(shape, lambda i: (0,) * len(shape), pipeline_mode=pl.Buffered(1))

    blk = pl.BlockSpec((T, D), lambda i: (i, 0))
    in_specs = [res((S, D)), res((D, D)), res((D, DH)), res((D, DH)), res((D, D)),
                res((D, F)), res((D, F)), res((F, D)), blk]
    out_specs = [blk, res((S, D)), res((D, D)), res((D, DH)), res((D, DH)), res((D, D)),
                 res((D, F)), res((D, F)), res((F, D))]
    sds = jax.ShapeDtypeStruct
    out_shape = [sds((S, D), bf), sds((S, D), bf), sds((D, D), bf), sds((D, DH), bf), sds((D, DH), bf),
                 sds((D, D), bf), sds((D, F), bf), sds((D, F), bf), sds((F, D), bf)]
    u32 = jnp.uint32
    VM = pltpu.VMEM
    scratch = [
        VM((S, D), bf),
        VM((D, D), bf),
        VM((16, S), u32),
        VM((16, S), u32),
        VM((H * NQ, 64, 128), u32),
        VM((D // 2, T), u32),
        VM((H * NQ, 64, 128), u32),
        VM((D // 2, T), u32),
        VM((H * NQ, 64, S), u32),
        VM((hpi_b * NQ * NC, 64, KC), u32),
        VM((H * NQ, 16, 128), f32),
        VM((H * NQ, 1, 128), f32),
        VM((H * NQ, 16, 128), f32),
        VM((16, S), f32),
        VM((16, S), f32),
        VM((D, D), f32),
        VM((D, D), f32),
        VM((D, F), f32),
        VM((D, F), f32),
        VM((F, D), f32),
        VM((S, D), f32),
        pltpu.SMEM((1,), f32),
    ]
    outs = pl.pallas_call(
        _make_kernel(T, hpi_f, hpi_b, lag_f, lag_b),
        grid=(S // T,),
        in_specs=in_specs,
        out_specs=out_specs,
        out_shape=out_shape,
        scratch_shapes=scratch,
        compiler_params=pltpu.CompilerParams(
            dimension_semantics=("arbitrary",),
            vmem_limit_bytes=120 * 1024 * 1024),
    )(x2, A_wq, A_wk, A_wv, A_wo, B_w1, B_w3, B_w2, g2)
    out, dx, dwq, dwk, dwv, dwo, dw1, dw3, dw2 = outs
    return (out.reshape(1, S, D), dx.reshape(1, S, D), dwq, dwk, dwv, dwo, dw1, dw3, dw2)


@jax.jit
def pallas_sequential_preLN__grouped_kv_mqa__glu_gated_swiglu__prompt_kernel(
    A_x: jax.Array,
    A_wq: jax.Array,
    A_wk: jax.Array,
    A_wv: jax.Array,
    A_wo: jax.Array,
    B_x: jax.Array,
    B_w1: jax.Array,
    B_w3: jax.Array,
    B_w2: jax.Array,
    grad_out: jax.Array,
):
    del B_x
    return _call(A_x, A_wq, A_wk, A_wv, A_wo, B_w1, B_w3, B_w2, grad_out)
```
